```python
import os as _os
_os.environ.setdefault("JAX_PLATFORMS", "cpu")
import jax
import jax.numpy as jnp

def _softmax(x, axis=-1):
    return jax.nn.softmax(x, axis=axis)
def _gelu(x):
    return jax.nn.gelu(x, approximate=True)
def _silu(x):
    return jax.nn.silu(x)
def _sigmoid(x):
    return jax.nn.sigmoid(x)
def _layernorm(x, axis=-1, eps=1e-5):
    m = jnp.mean(x, axis=axis, keepdims=True)
    v = jnp.var(x, axis=axis, keepdims=True)
    return (x - m) / jnp.sqrt(v + eps)
def _scatter_add(tgt, idx, src, axis=0):
    return tgt.at[idx].add(src)
def _segment_sum(src, seg, n):
    return jax.ops.segment_sum(src, seg, n)
class _Rng:
    def __init__(self, key):
        self._k = key
    def _next(self):
        self._k, sub = jax.random.split(self._k)
        return sub
    def normal(self, shape):
        return jax.random.normal(self._next(), shape, dtype=jnp.bfloat16)
    def randint(self, lo, hi, shape):
        return jax.random.randint(self._next(), shape, lo, hi, dtype=jnp.int32)
    def uniform(self, shape, lo=0.0, hi=1.0):
        return jax.random.uniform(self._next(), shape, jnp.bfloat16, lo, hi)
    def permutation(self, n):
        return jax.random.permutation(self._next(), n)


kernel_name = 'gated_mix__mha_block__mha_block__prompt'

def setup_inputs():
    _rng = _Rng(jax.random.key(int.from_bytes(__import__("os").urandom(4), "little")))
    _w = (lambda a: (lambda t: t.astype(jnp.bfloat16) if jnp.issubdtype(t.dtype, jnp.floating) else t)(jnp.asarray(a)))
    def _A_setup():
        B, S, D, H = 1, 2048, 448, 16
        return {
            "x": _w((lambda *s: _rng.normal(s) * 0.05)(B, S, D)),
            "wqkv": _w((lambda *s: _rng.normal(s) * 0.4)(D, 3 * D)),
            "wo": _w((lambda *s: _rng.normal(s) * 0.05)(D, D)),
        }
    _A_in = _A_setup()

    def _B_setup():
        B, S, D, H = 1, 2048, 448, 16
        return {
            "x": _w((lambda *s: _rng.normal(s) * 0.05)(B, S, D)),
            "wqkv": _w((lambda *s: _rng.normal(s) * 0.4)(D, 3 * D)),
            "wo": _w((lambda *s: _rng.normal(s) * 0.05)(D, D)),
        }
    _B_in = _B_setup()

    return {
        "A_x": _A_in["x"],
        "A_wqkv": _A_in["wqkv"],
        "A_wo": _A_in["wo"],
        "B_x": _B_in["x"],
        "B_wqkv": _B_in["wqkv"],
        "B_wo": _B_in["wo"],
        "gate_w": _w((lambda *s: _rng.normal(s) * 0.05)(448) * 16.0),
    }

def reference(A_x, A_wqkv, A_wo, B_x, B_wqkv, B_wo, gate_w):
    def _A_ref(x, wqkv, wo):
        B, S, D = x.shape
        H = 16
        Dh = D // H
        qkv = (lambda x, *d: x.transpose(*d))((x @ wqkv).reshape(B, S, 3, H, Dh), 2, 0, 3, 1, 4)
        q, k, v = qkv[0], qkv[1], qkv[2]
        scores = jnp.einsum("bhqd,bhkd->bhqk", q, k) * (Dh ** -0.5)
        p = _softmax(scores, axis=-1)
        o = jnp.einsum("bhqk,bhkd->bhqd", p, v)
        return (lambda x, *d: x.transpose(*d))(o, 0, 2, 1, 3).reshape(B, S, D) @ wo

    def _B_ref(x, wqkv, wo):
        B, S, D = x.shape
        H = 16
        Dh = D // H
        qkv = (lambda x, *d: x.transpose(*d))((x @ wqkv).reshape(B, S, 3, H, Dh), 2, 0, 3, 1, 4)
        q, k, v = qkv[0], qkv[1], qkv[2]
        scores = jnp.einsum("bhqd,bhkd->bhqk", q, k) * (Dh ** -0.5)
        p = _softmax(scores, axis=-1)
        o = jnp.einsum("bhqk,bhkd->bhqd", p, v)
        return (lambda x, *d: x.transpose(*d))(o, 0, 2, 1, 3).reshape(B, S, D) @ wo

    x = A_x
    g = _sigmoid((x * gate_w).sum(-1, keepdims=True))
    a = _A_ref(x, A_wqkv, A_wo)
    b = _B_ref(x, B_wqkv, B_wo)
    return g * a + (1 - g) * b
```

```python
import functools, math
import jax, jax.numpy as jnp, numpy as np
from jax import lax
from jax.experimental import pallas as pl
from jax.experimental.pallas import tpu as pltpu

H = 16; DH = 28; DP = 32; W = 512; CK = 128
F32 = jnp.float32; BF16 = jnp.bfloat16
GR = 16


def _kernel(x_hbm, wa_hbm, wb_hbm, woa_hbm, wob_hbm, gw_hbm, o_hbm,
            x_scr, w_scr, wo_scr, gw_scr, wt_scr, wot_scr, k_scr, qt_scr, vt_scr, g_scr,
            s0, s1, m_scr, acc_scr, out_scr, sem_x, sem_w, sem_wo, sem_g, sem_o, *, S, D, BQ, LAG):
    c_scale = (DH ** -0.5) * math.log2(math.e)
    nt = (((1,), (1,)), ((), ()))
    NCH = S // W
    NS = BQ // W
    NQ = S // BQ
    NH = 2 * H
    nc = S // CK
    w_hbm = (wa_hbm, wb_hbm); wo_hbm = (woa_hbm, wob_hbm)

    def x_copy(n):
        return pltpu.make_async_copy(x_hbm.at[:, pl.ds(n * W, W)], x_scr.at[n], sem_x.at[n])
    def w_copy(b):
        return pltpu.make_async_copy(w_hbm[b], w_scr.at[b], sem_w.at[b])
    def wo_copy(b):
        return pltpu.make_async_copy(wo_hbm[b], wo_scr.at[b], sem_wo.at[b])
    g_copy = pltpu.make_async_copy(gw_hbm, gw_scr, sem_g)

    w_copy(0).start(); g_copy.start()
    for n in range(NCH): x_copy(n).start()
    w_copy(1).start()
    wo_copy(0).start(); wo_copy(1).start()

    def proj_body(i, _):
        b = i // NCH; n = i % NCH

        @pl.when(n == 0)
        def _():
            @pl.when(b == 0)
            def _():
                w_copy(0).wait(); g_copy.wait()
            @pl.when(b == 1)
            def _():
                w_copy(1).wait()
            wt_scr[0:3 * D, :] = w_scr[b].T
            wt_scr[3 * D:3 * D + GR, :] = jnp.broadcast_to(gw_scr[...], (GR, D))

        for nn in range(NCH):
            @pl.when(i == nn)
            def _():
                x_copy(nn).wait()

        r = jnp.dot(wt_scr[...], x_scr[n], preferred_element_type=F32)
        z4 = jnp.zeros((DP - DH, W), F32)
        ones4 = jnp.where(lax.broadcasted_iota(jnp.int32, (DP - DH, W), 0) == 0, 1.0, 0.0).astype(F32)
        for h in range(H):
            q = r[h * DH:(h + 1) * DH] * c_scale
            qt_scr[b * H + h, n] = jnp.concatenate([q, z4], axis=0).astype(BF16)
            k = r[D + h * DH:D + (h + 1) * DH]
            k_scr[b * H + h, n] = jnp.concatenate([k, z4], axis=0).T.astype(BF16)
            v = r[2 * D + h * DH:2 * D + (h + 1) * DH]
            vt_scr[b * H + h, n] = jnp.concatenate([v, ones4], axis=0).astype(BF16)
        g_scr[b, n] = jax.nn.sigmoid(r[3 * D:3 * D + 8])
        return 0
    lax.fori_loop(0, 2 * NCH, proj_body, 0)

    wo_copy(0).wait(); wo_copy(1).wait()
    def wo_body(b, _):
        wo = wo_scr[b].astype(F32)
        z4 = jnp.zeros((DP - DH, D), F32)
        wop = jnp.concatenate([jnp.concatenate([wo[h * DH:(h + 1) * DH], z4], axis=0) for h in range(H)], axis=0)
        wot_scr[b] = wop.T.astype(BF16)
        return 0
    lax.fori_loop(0, 2, wo_body, 0)

    def a_chunk(h, q, c, m, sbuf, sub):
        kc = k_scr[h, c * CK // W, pl.ds(c * CK % W, CK), :]
        s = jnp.dot(kc, q, preferred_element_type=F32)
        sbuf[sub, pl.ds(c * CK, CK), :] = s
        mc = jnp.max(s.reshape(CK // 8, 8, W), axis=0)
        return mc if m is None else jnp.maximum(m, mc)

    def b_chunk(h, c, m, acc, sbuf, sub):
        s = sbuf[sub, pl.ds(c * CK, CK), :]
        p = jnp.exp2(s.reshape(CK // 8, 8, W) - m[None]).reshape(CK, W).astype(BF16)
        v = vt_scr[h, c * CK // W, :, pl.ds(c * CK % W, CK)]
        o = jnp.dot(v, p, preferred_element_type=F32)
        return o if acc is None else acc + o

    total = NH * NQ

    def unit(u):
        return u % NH, (u // NH) * NS

    def step(u, cur, nxt):
        hn, qn = unit(jnp.minimum(u + 1, total - 1))
        h, q0 = unit(u)
        m_cur = jnp.broadcast_to(jnp.max(m_scr[...], axis=0, keepdims=True), (8, BQ))
        ms = [None] * NS; accs = [None] * NS
        qs = [qt_scr[hn, qn + sub] for sub in range(NS)]
        for t in range(NS * nc + LAG):
            if t < NS * nc:
                sub, c = divmod(t, nc)
                ms[sub] = a_chunk(hn, qs[sub], c, ms[sub], nxt, sub)
                if c == nc - 1:
                    m_scr[:, pl.ds(sub * W, W)] = ms[sub]
            if t >= LAG:
                sub, c = divmod(t - LAG, nc)
                accs[sub] = b_chunk(h, c, m_cur[:, sub * W:(sub + 1) * W], accs[sub], cur, sub)
                if c == nc - 1:
                    acc_scr[h, q0 + sub] = accs[sub]

    def a_only(sub, _):
        q = qt_scr[0, sub]
        m = None
        for c in range(nc):
            m = a_chunk(0, q, c, m, s0, sub)
        m_scr[:, pl.ds(pl.multiple_of(sub * W, W), W)] = m
        return 0
    lax.fori_loop(0, NS, a_only, 0)

    def body(u, _):
        for j in range(2):
            @pl.when(u % 2 == j)
            def _():
                step(u, *((s0, s1) if j == 0 else (s1, s0)))
        return 0
    lax.fori_loop(0, total - 1, body, 0)

    def b_only(sub, _):
        h, q0 = unit(total - 1)
        m8 = m_scr[:, pl.ds(pl.multiple_of(sub * W, W), W)]
        m_cur = jnp.broadcast_to(jnp.max(m8, axis=0, keepdims=True), (8, W))
        acc = None
        for c in range(nc):
            acc = b_chunk(h, c, m_cur, acc, s1, sub)
        acc_scr[h, q0 + sub] = acc
        return 0
    lax.fori_loop(0, NS, b_only, 0)

    def out_copy(n):
        return pltpu.make_async_copy(out_scr.at[n], o_hbm.at[:, pl.ds(n * W, W)], sem_o.at[n])

    def out_body(n, _):
        g = g_scr[0, n][0:1, :]
        acc_t = None
        for b in range(2):
            gg = g if b == 0 else 1.0 - g
            parts = []
            for h in range(H):
                a = acc_scr[b * H + h, n]
                parts.append((a * (gg / a[DH:DH + 1])).astype(BF16))
            ot = jnp.concatenate(parts, axis=0)
            t = jnp.dot(wot_scr[b], ot, preferred_element_type=F32)
            acc_t = t if acc_t is None else acc_t + t
        out_scr[n] = acc_t.astype(out_scr.dtype)
        out_copy(n).start()
        return 0
    lax.fori_loop(0, NCH, out_body, 0)
    for n in range(NCH):
        out_copy(n).wait()


def make(BQ=2048, LAG=1):
    @jax.jit
    def f(A_x, A_wqkv, A_wo, B_x, B_wqkv, B_wo, gate_w):
        _, S, D = A_x.shape
        NCH = S // W
        any_spec = pl.BlockSpec(memory_space=pltpu.HBM)
        out = pl.pallas_call(
            functools.partial(_kernel, S=S, D=D, BQ=BQ, LAG=LAG),
            out_shape=jax.ShapeDtypeStruct((D, S), A_x.dtype),
            in_specs=[any_spec] * 6,
            out_specs=any_spec,
            scratch_shapes=[
                pltpu.VMEM((NCH, D, W), BF16),
                pltpu.VMEM((2, D, 3 * D), BF16),
                pltpu.VMEM((2, D, D), BF16),
                pltpu.VMEM((1, D), BF16),
                pltpu.VMEM((3 * D + GR, D), BF16),
                pltpu.VMEM((2, D, H * DP), BF16),
                pltpu.VMEM((2 * H, NCH, W, DP), BF16),
                pltpu.VMEM((2 * H, NCH, DP, W), BF16),
                pltpu.VMEM((2 * H, NCH, DP, W), BF16),
                pltpu.VMEM((2, NCH, 8, W), F32),
                pltpu.VMEM((BQ // W, S, W), F32),
                pltpu.VMEM((BQ // W, S, W), F32),
                pltpu.VMEM((8, BQ), F32),
                pltpu.VMEM((2 * H, NCH, DP, W), F32),
                pltpu.VMEM((NCH, D, W), BF16),
                pltpu.SemaphoreType.DMA((NCH,)),
                pltpu.SemaphoreType.DMA((2,)),
                pltpu.SemaphoreType.DMA((2,)),
                pltpu.SemaphoreType.DMA(()),
                pltpu.SemaphoreType.DMA((NCH,)),
            ],
            compiler_params=pltpu.CompilerParams(vmem_limit_bytes=110 * 1024 * 1024),
        )(A_x[0].T, A_wqkv, B_wqkv, A_wo, B_wo, gate_w.reshape(1, D))
        return out.T[None]
    return f


_impl = make(BQ=2048)


def pallas_gated_mix__mha_block__mha_block__prompt_kernel(A_x, A_wqkv, A_wo, B_x, B_wqkv, B_wo, gate_w):
    return _impl(A_x, A_wqkv, A_wo, B_x, B_wqkv, B_wo, gate_w)
```

```python
import functools, math
import jax, jax.numpy as jnp, numpy as np
from jax import lax
from jax.experimental import pallas as pl
from jax.experimental.pallas import tpu as pltpu

H = 16; DH = 28; DP = 32; W = 512; CK = 128
F32 = jnp.float32; BF16 = jnp.bfloat16
GR = 16


def _kernel(x_hbm, wa_hbm, wb_hbm, woa_hbm, wob_hbm, gw_hbm, o_hbm,
            x_scr, w_scr, wo_scr, gw_scr, k_scr, qt_scr, vt_scr, g_scr,
            s_scr, m_scr, acc_scr, out_scr, sem_x, sem_w, sem_wo, sem_g, sem_o, *, S, D, BQ, LAG, HPS, ORD, KZ, PU, OU, GL):
    c_scale = (DH ** -0.5) * math.log2(math.e)
    tn = (((0,), (0,)), ((), ()))
    NCH = S // W
    NS = BQ // W
    NQ = S // BQ
    NH = 2 * H
    nc = S // CK
    w_hbm = (wa_hbm, wb_hbm); wo_hbm = (woa_hbm, wob_hbm)

    def x_copy(i):
        return pltpu.make_async_copy(x_hbm.at[:, pl.ds(pl.multiple_of((i % NCH) * W, W), W)], x_scr.at[i], sem_x.at[i])
    def w_copy(b):
        return pltpu.make_async_copy(w_hbm[b], w_scr.at[b], sem_w.at[b])
    def wo_copy(b):
        return pltpu.make_async_copy(wo_hbm[b], wo_scr.at[pl.ds(b * D, D), :], sem_wo.at[b])
    g_copy = pltpu.make_async_copy(gw_hbm, gw_scr, sem_g)

    w_copy(0).start(); g_copy.start()
    for i in range(NCH): x_copy(i).start()
    w_copy(1).start()
    for i in range(NCH, 2 * NCH): x_copy(i).start()
    wo_copy(0).start(); wo_copy(1).start()

    def proj_body(it, _):
        i0 = it * PU
        @pl.when(i0 == 0)
        def _():
            w_copy(0).wait(); g_copy.wait()
        @pl.when(i0 == NCH)
        def _():
            w_copy(1).wait()
        for j in range(PU):
            proj_chunk(i0 + j)
        return 0

    def proj_chunk(i):
        b = i // NCH; n = i % NCH
        x_copy(i).wait()
        xs = x_scr[i]
        r = lax.dot_general(w_scr[b], xs, tn, preferred_element_type=F32)
        z4 = jnp.zeros((DP - DH, W), F32)
        ones4 = jnp.where(lax.broadcasted_iota(jnp.int32, (DP - DH, W), 0) == 0, 1.0, 0.0).astype(F32)
        for h in range(H):
            q = r[h * DH:(h + 1) * DH] * c_scale
            qt_scr[b * H + h, n] = jnp.concatenate([q, z4], axis=0).astype(BF16)
            k = r[D + h * DH:D + (h + 1) * DH]
            zk = jnp.zeros(((128 if KZ else DP) - DH, W), F32)
            k_scr[b * H + h, n] = jnp.concatenate([k, zk], axis=0).T.astype(BF16)
            v = r[2 * D + h * DH:2 * D + (h + 1) * DH]
            vt_scr[b * H + h, n] = jnp.concatenate([v, ones4], axis=0).astype(BF16)
    lax.fori_loop(0, 2 * NCH // PU, proj_body, 0)

    wo_copy(0).wait(); wo_copy(1).wait()

    def gate(n):
        xs = x_scr[n].astype(F32)
        gs = jnp.sum((xs * gw_scr[...].astype(F32)).reshape(D // 8, 8, W), axis=0)
        g_scr[n] = jax.nn.sigmoid(jnp.broadcast_to(jnp.sum(gs, axis=0, keepdims=True), (8, W)))

    def a_chunk(h, q, c, m, sbuf, sub):
        kc = k_scr[h, c * CK // W, pl.ds(c * CK % W, CK), 0:DP]
        s = jnp.dot(kc, q, preferred_element_type=F32)
        sbuf[sub, pl.ds(c * CK, CK), :] = s
        mc = jnp.max(s.reshape(CK // 8, 8, W), axis=0)
        return mc if m is None else jnp.maximum(m, mc)

    def b_chunk(h, c, m, acc, sbuf, sub):
        s = sbuf[sub, pl.ds(c * CK, CK), :]
        p = jnp.exp2(s.reshape(CK // 8, 8, W) - m[None]).reshape(CK, W).astype(BF16)
        v = vt_scr[h, c * CK // W, :, pl.ds(c * CK % W, CK)]
        o = jnp.dot(v, p, preferred_element_type=F32)
        return o if acc is None else acc + o

    total = NH * NQ

    def unit(u):
        return u % NH, (u // NH) * NS

    def step(u):
        hn, qn = unit(u + 1)
        h, q0 = unit(u)
        m_cur = jnp.broadcast_to(jnp.max(m_scr[...], axis=0, keepdims=True), (8, BQ))
        ms = [None] * NS; accs = [None] * NS
        qs = [qt_scr[hn, qn + sub] for sub in range(NS)]
        for t in range(NS * nc + LAG):
            if t < NS * nc:
                sub, c = divmod(t, nc) if ORD == 0 else divmod(t, NS)[::-1]
                accs[sub] = b_chunk(h, c, m_cur[:, sub * W:(sub + 1) * W], accs[sub], s_scr, sub)
                if c == nc - 1:
                    acc_scr[h, q0 + sub] = accs[sub]
            if t >= LAG:
                sub, c = divmod(t - LAG, nc) if ORD == 0 else divmod(t - LAG, NS)[::-1]
                ms[sub] = a_chunk(hn, qs[sub], c, ms[sub], s_scr, sub)
                if c == nc - 1:
                    m_scr[:, pl.ds(sub * W, W)] = ms[sub]

    def a_only(sub, _):
        q = qt_scr[0, sub]
        m = None
        for c in range(nc):
            m = a_chunk(0, q, c, m, s_scr, sub)
        m_scr[:, pl.ds(pl.multiple_of(sub * W, W), W)] = m
        if GL == 'a':
            for j in range(NCH // NS): gate(sub * (NCH // NS) + j)
        return 0
    lax.fori_loop(0, NS, a_only, 0)

    def body(i, _):
        for j in range(HPS):
            step(i * HPS + j)
        return 0
    lax.fori_loop(0, (total - 1) // HPS, body, 0)
    for j in range((total - 1) % HPS):
        step((total - 1) // HPS * HPS + j)

    def b_only(sub, _):
        h, q0 = unit(total - 1)
        m8 = m_scr[:, pl.ds(pl.multiple_of(sub * W, W), W)]
        m_cur = jnp.broadcast_to(jnp.max(m8, axis=0, keepdims=True), (8, W))
        acc = None
        for c in range(nc):
            acc = b_chunk(h, c, m_cur, acc, s_scr, sub)
        acc_scr[h, q0 + sub] = acc
        if GL == 'b':
            for j in range(NCH // NS): gate(sub * (NCH // NS) + j)
        return 0
    lax.fori_loop(0, NS, b_only, 0)

    def out_copy(n):
        return pltpu.make_async_copy(out_scr.at[n], o_hbm.at[:, pl.ds(n * W, W)], sem_o.at[n])

    def out_body(n, _):
        g = g_scr[n][0:1, :]
        parts = []
        for hh in range(2 * H):
            a = acc_scr[hh, n]
            gg = g if hh < H else 1.0 - g
            parts.append(a[0:DH] * (gg / a[DH:DH + 1]))
        ot = jnp.concatenate(parts, axis=0).astype(BF16)
        out_scr[n] = lax.dot_general(wo_scr[...], ot, tn, preferred_element_type=F32).astype(out_scr.dtype)
        out_copy(n).start()
        return 0
    lax.fori_loop(0, NCH, out_body, 0, unroll=OU)
    for n in range(NCH):
        out_copy(n).wait()


def make(BQ=1024, LAG=0, HPS=7, ORD=1, KZ=1, PU=1, OU=4, GL='b'):
    @jax.jit
    def f(A_x, A_wqkv, A_wo, B_x, B_wqkv, B_wo, gate_w):
        _, S, D = A_x.shape
        NCH = S // W
        any_spec = pl.BlockSpec(memory_space=pltpu.HBM)
        out = pl.pallas_call(
            functools.partial(_kernel, S=S, D=D, BQ=BQ, LAG=LAG, HPS=HPS, ORD=ORD, KZ=KZ, PU=PU, OU=OU, GL=GL),
            out_shape=jax.ShapeDtypeStruct((D, S), A_x.dtype),
            in_specs=[any_spec] * 6,
            out_specs=any_spec,
            scratch_shapes=[
                pltpu.VMEM((2 * NCH, D, W), BF16),
                pltpu.VMEM((2, D, 3 * D), BF16),
                pltpu.VMEM((2 * D, D), BF16),
                pltpu.VMEM((D, 1), BF16),
                pltpu.VMEM((2 * H, NCH, W, 128 if KZ else DP), BF16),
                pltpu.VMEM((2 * H, NCH, DP, W), BF16),
                pltpu.VMEM((2 * H, NCH, DP, W), BF16),
                pltpu.VMEM((NCH, 8, W), F32),
                pltpu.VMEM((BQ // W, S, W), F32),
                pltpu.VMEM((8, BQ), F32),
                pltpu.VMEM((2 * H, NCH, DP, W), F32),
                pltpu.VMEM((NCH, D, W), BF16),
                pltpu.SemaphoreType.DMA((2 * NCH,)),
                pltpu.SemaphoreType.DMA((2,)),
                pltpu.SemaphoreType.DMA((2,)),
                pltpu.SemaphoreType.DMA(()),
                pltpu.SemaphoreType.DMA((NCH,)),
            ],
            compiler_params=pltpu.CompilerParams(vmem_limit_bytes=110 * 1024 * 1024),
        )(A_x[0].T, A_wqkv, B_wqkv, A_wo, B_wo, gate_w.reshape(D, 1))
        return out.T[None]
    return f


_impl = make(GL='a')


def pallas_gated_mix__mha_block__mha_block__prompt_kernel(A_x, A_wqkv, A_wo, B_x, B_wqkv, B_wo, gate_w):
    return _impl(A_x, A_wqkv, A_wo, B_x, B_wqkv, B_wo, gate_w)
```

```python
import functools, math
import jax, jax.numpy as jnp, numpy as np
from jax import lax
from jax.experimental import pallas as pl
from jax.experimental.pallas import tpu as pltpu

H = 16; DH = 28; DP = 32; W = 512; CK = 128
F32 = jnp.float32; BF16 = jnp.bfloat16
GR = 16


def _kernel(x_hbm, wa_hbm, wb_hbm, woa_hbm, wob_hbm, gw_hbm, o_hbm,
            x_scr, w_scr, wo_scr, gw_scr, gcol_scr, k_scr, qt_scr, vt_scr, g_scr,
            s_scr, m_scr, acc_scr, out_scr, sem_x, sem_w, sem_wo, sem_g, sem_o, *, S, D, BQ, LAG, HPS, ORD, KZ, PU, OU, GL, AU):
    c_scale = (DH ** -0.5) * math.log2(math.e)
    tn = (((0,), (0,)), ((), ()))
    NCH = S // W
    NS = BQ // W
    NQ = S // BQ
    NH = 2 * H
    nc = S // CK
    w_hbm = (wa_hbm, wb_hbm); wo_hbm = (woa_hbm, wob_hbm)

    def x_copy(i):
        return pltpu.make_async_copy(x_hbm.at[:, pl.ds(pl.multiple_of((i % NCH) * W, W), W)], x_scr.at[i], sem_x.at[i])
    def w_copy(b):
        return pltpu.make_async_copy(w_hbm[b], w_scr.at[b], sem_w.at[b])
    def wo_copy(b):
        return pltpu.make_async_copy(wo_hbm[b], wo_scr.at[pl.ds(b * D, D), :], sem_wo.at[b])
    g_copy = pltpu.make_async_copy(gw_hbm, gw_scr, sem_g)

    w_copy(0).start(); g_copy.start()
    for i in range(PU): x_copy(i).start()
    w_copy(0).wait(); g_copy.wait()
    for i in range(PU): x_copy(i).wait()
    for i in range(PU, NCH): x_copy(i).start()
    w_copy(1).start(); wo_copy(0).start(); wo_copy(1).start()

    def proj_body(it, _):
        i0 = it * PU
        @pl.when((i0 > 0) & (i0 < NCH))
        def _():
            for j in range(PU): x_copy(i0 + j).wait()
        @pl.when(i0 == NCH)
        def _():
            w_copy(1).wait()
        for j in range(PU):
            proj_chunk(i0 + j)
        return 0

    def proj_chunk(i):
        b = i // NCH; n = i % NCH
        xs = x_scr[n]
        r = lax.dot_general(w_scr[b], xs, tn, preferred_element_type=F32)
        z4 = jnp.zeros((DP - DH, W), F32)
        ones4 = jnp.where(lax.broadcasted_iota(jnp.int32, (DP - DH, W), 0) == 0, 1.0, 0.0).astype(F32)
        for h in range(H):
            q = r[h * DH:(h + 1) * DH] * c_scale
            qt_scr[b * H + h, n] = jnp.concatenate([q, z4], axis=0).astype(BF16)
            k = r[D + h * DH:D + (h + 1) * DH]
            zk = jnp.zeros(((128 if KZ else DP) - DH, W), F32)
            k_scr[b * H + h, n] = jnp.concatenate([k, zk], axis=0).T.astype(BF16)
            v = r[2 * D + h * DH:2 * D + (h + 1) * DH]
            vt_scr[b * H + h, n] = jnp.concatenate([v, ones4], axis=0).astype(BF16)
    lax.fori_loop(0, 2 * NCH // PU, proj_body, 0)

    wo_copy(0).wait(); wo_copy(1).wait()

    def gate(n):
        gc = gcol_scr[...]
        for j in range(W // 128):
            xs = x_scr[n, :, j * 128:(j + 1) * 128].astype(F32)
            gs = jnp.sum((xs * gc).reshape(D // 8, 8, 128), axis=0)
            g_scr[n, :, j * 128:(j + 1) * 128] = jax.nn.sigmoid(jnp.broadcast_to(jnp.sum(gs, axis=0, keepdims=True), (8, 128)))

    gcol_scr[...] = jnp.broadcast_to(gw_scr[...].astype(F32).reshape(1, D), (128, D)).T
    def a_chunk(h, q, c, m, sbuf, sub):
        kc = k_scr[h, c * CK // W, pl.ds(c * CK % W, CK), 0:DP]
        s = jnp.dot(kc, q, preferred_element_type=F32)
        sbuf[sub, pl.ds(c * CK, CK), :] = s
        mc = jnp.max(s.reshape(CK // 8, 8, W), axis=0)
        return mc if m is None else jnp.maximum(m, mc)

    def b_chunk(h, c, m, acc, sbuf, sub):
        s = sbuf[sub, pl.ds(c * CK, CK), :]
        p = jnp.exp2(s.reshape(CK // 8, 8, W) - m[None]).reshape(CK, W).astype(BF16)
        v = vt_scr[h, c * CK // W, :, pl.ds(c * CK % W, CK)]
        o = jnp.dot(v, p, preferred_element_type=F32)
        return o if acc is None else acc + o

    total = NH * NQ

    def unit(u):
        return u % NH, (u // NH) * NS

    order = [(sub, g * ORD + j) for g in range(nc // ORD) for sub in range(NS) for j in range(ORD)]

    def step(u):
        hn, qn = unit(u + 1)
        h, q0 = unit(u)
        m_cur = jnp.broadcast_to(jnp.max(m_scr[...], axis=0, keepdims=True), (8, BQ))
        ms = [None] * NS; accs = [None] * NS
        qs = [qt_scr[hn, qn + sub] for sub in range(NS)]
        for t in range(NS * nc + LAG):
            if t < NS * nc:
                sub, c = order[t]
                accs[sub] = b_chunk(h, c, m_cur[:, sub * W:(sub + 1) * W], accs[sub], s_scr, sub)
                if c == nc - 1:
                    acc_scr[h, q0 + sub] = accs[sub]
            if t >= LAG:
                sub, c = order[t - LAG]
                ms[sub] = a_chunk(hn, qs[sub], c, ms[sub], s_scr, sub)
                if c == nc - 1:
                    m_scr[:, pl.ds(sub * W, W)] = ms[sub]

    def a_only(sub, _):
        q = qt_scr[0, sub]
        m = None
        for c in range(nc):
            m = a_chunk(0, q, c, m, s_scr, sub)
        m_scr[:, pl.ds(pl.multiple_of(sub * W, W), W)] = m
        if GL == 'a':
            for j in range(NCH // NS): gate(sub * (NCH // NS) + j)
        return 0
    lax.fori_loop(0, NS, a_only, 0, unroll=AU)

    def body(i, _):
        for j in range(HPS):
            step(i * HPS + j)
        return 0
    lax.fori_loop(0, (total - 1) // HPS, body, 0)
    for j in range((total - 1) % HPS):
        step((total - 1) // HPS * HPS + j)

    def b_only(sub, _):
        h, q0 = unit(total - 1)
        m8 = m_scr[:, pl.ds(sub * W, W)]
        m_cur = jnp.broadcast_to(jnp.max(m8, axis=0, keepdims=True), (8, W))
        acc = None
        for c in range(nc):
            acc = b_chunk(h, c, m_cur, acc, s_scr, sub)
        acc_scr[h, q0 + sub] = acc
        if GL == 'b':
            for j in range(NCH // NS): gate(sub * (NCH // NS) + j)
        return 0

    def out_copy(n):
        return pltpu.make_async_copy(out_scr.at[n], o_hbm.at[:, pl.ds(n * W, W)], sem_o.at[n])

    def out_body(n, _):
        g = g_scr[n][0:1, :]
        parts = []
        for hh in range(2 * H):
            a = acc_scr[hh, n]
            gg = g if hh < H else 1.0 - g
            parts.append(a[0:DH] * (gg / a[DH:DH + 1]))
        ot = jnp.concatenate(parts, axis=0).astype(BF16)
        out_scr[n] = lax.dot_general(wo_scr[...], ot, tn, preferred_element_type=F32).astype(out_scr.dtype)
        out_copy(n).start()
        return 0
    if OU == 0:
        for sub in range(NS): b_only(sub, 0)
        for n in range(NCH): out_body(n, 0)
    elif OU == 1:
        for n in range(NCH - NS): out_body(n, 0)
        for sub in range(NS):
            b_only(sub, 0); out_body(NCH - NS + sub, 0)
    else:
        for sub in range(NS):
            b_only(sub, 0); out_body(sub, 0)
        for n in range(NS, NCH): out_body(n, 0)
    for n in range(NCH):
        out_copy(n).wait()


def make(BQ=1024, LAG=0, HPS=7, ORD=1, KZ=1, PU=2, OU=2, GL='a', AU=1):
    @jax.jit
    def f(A_x, A_wqkv, A_wo, B_x, B_wqkv, B_wo, gate_w):
        _, S, D = A_x.shape
        NCH = S // W
        any_spec = pl.BlockSpec(memory_space=pltpu.HBM)
        out = pl.pallas_call(
            functools.partial(_kernel, S=S, D=D, BQ=BQ, LAG=LAG, HPS=HPS, ORD=ORD, KZ=KZ, PU=PU, OU=OU, GL=GL, AU=AU),
            out_shape=jax.ShapeDtypeStruct((D, S), A_x.dtype),
            in_specs=[any_spec] * 6,
            out_specs=any_spec,
            scratch_shapes=[
                pltpu.VMEM((NCH, D, W), BF16),
                pltpu.VMEM((2, D, 3 * D), BF16),
                pltpu.VMEM((2 * D, D), BF16),
                pltpu.VMEM((D,), BF16),
                pltpu.VMEM((D, 128), F32),
                pltpu.VMEM((2 * H, NCH, W, 128 if KZ else DP), BF16),
                pltpu.VMEM((2 * H, NCH, DP, W), BF16),
                pltpu.VMEM((2 * H, NCH, DP, W), BF16),
                pltpu.VMEM((NCH, 8, W), F32),
                pltpu.VMEM((BQ // W, S, W), F32),
                pltpu.VMEM((8, BQ), F32),
                pltpu.VMEM((2 * H, NCH, DP, W), F32),
                pltpu.VMEM((NCH, D, W), BF16),
                pltpu.SemaphoreType.DMA((NCH,)),
                pltpu.SemaphoreType.DMA((2,)),
                pltpu.SemaphoreType.DMA((2,)),
                pltpu.SemaphoreType.DMA(()),
                pltpu.SemaphoreType.DMA((NCH,)),
            ],
            compiler_params=pltpu.CompilerParams(vmem_limit_bytes=110 * 1024 * 1024),
        )(A_x[0].T, A_wqkv, B_wqkv, A_wo, B_wo, gate_w)
        return out.T[None]
    return f


_impl = make(ORD=2)


def pallas_gated_mix__mha_block__mha_block__prompt_kernel(A_x, A_wqkv, A_wo, B_x, B_wqkv, B_wo, gate_w):
    return _impl(A_x, A_wqkv, A_wo, B_x, B_wqkv, B_wo, gate_w)
```

```python
import functools
import math

import jax
import jax.numpy as jnp
from jax import lax
from jax.experimental import pallas as pl
from jax.experimental.pallas import tpu as pltpu

H = 16
DP = 32
W = 512
CK = 128
BQ = 1024
GRP = 2
UNROLL = 7
MS = 256
F32 = jnp.float32
BF16 = jnp.bfloat16


def _kernel(x_hbm, wa_hbm, wb_hbm, woa_hbm, wob_hbm, gw_hbm, o_hbm,
            x_scr, w_scr, wo_scr, gw_scr, gcol_scr, k_scr, qt_scr, vt_scr, g_scr,
            s_scr, m_scr, acc_scr, out_scr, sem_x, sem_w, sem_wo, sem_g, sem_o, *, S, D):
    DH = D // H
    NCH = S // W
    NS = BQ // W
    NH = 2 * H
    NC = S // CK
    total = NH * (S // BQ)
    q_scale = (DH ** -0.5) * math.log2(math.e)
    tn = (((0,), (0,)), ((), ()))
    w_hbm = (wa_hbm, wb_hbm)
    wo_hbm = (woa_hbm, wob_hbm)

    def x_copy(n):
        return pltpu.make_async_copy(
            x_hbm.at[:, pl.ds(pl.multiple_of(n * W, W), W)], x_scr.at[n], sem_x.at[n])

    def w_copy(b):
        return pltpu.make_async_copy(w_hbm[b], w_scr.at[b], sem_w.at[b])

    def wo_copy(b):
        return pltpu.make_async_copy(wo_hbm[b], wo_scr.at[pl.ds(b * D, D), :], sem_wo.at[b])

    g_copy = pltpu.make_async_copy(gw_hbm, gw_scr, sem_g)

    w_copy(0).start(); g_copy.start(); x_copy(0).start(); x_copy(1).start()
    w_copy(0).wait(); g_copy.wait(); x_copy(0).wait(); x_copy(1).wait()
    for n in range(2, NCH):
        x_copy(n).start()
    w_copy(1).start(); wo_copy(0).start(); wo_copy(1).start()

    def proj_chunk(i):
        b = i // NCH
        n = i % NCH
        r = lax.dot_general(w_scr[b], x_scr[n], tn, preferred_element_type=F32)
        z4 = jnp.zeros((DP - DH, W), F32)
        zk = jnp.zeros((128 - DH, W), F32)
        ones4 = jnp.where(lax.broadcasted_iota(jnp.int32, (DP - DH, W), 0) == 0, 1.0, 0.0).astype(F32)
        for h in range(H):
            q = r[h * DH:(h + 1) * DH] * q_scale
            qt_scr[b * H + h, n] = jnp.concatenate([q, z4], axis=0).astype(BF16)
            k = r[D + h * DH:D + (h + 1) * DH]
            k_scr[b * H + h, n] = jnp.concatenate([k, zk], axis=0).T.astype(BF16)
            v = r[2 * D + h * DH:2 * D + (h + 1) * DH]
            vt_scr[b * H + h, n] = jnp.concatenate([v, ones4], axis=0).astype(BF16)

    def proj_body(it, carry):
        i0 = it * 2

        @pl.when((i0 > 0) & (i0 < NCH))
        def _():
            x_copy(i0).wait()
            x_copy(i0 + 1).wait()

        @pl.when(i0 == NCH)
        def _():
            w_copy(1).wait()

        proj_chunk(i0)
        proj_chunk(i0 + 1)
        return carry

    lax.fori_loop(0, NCH, proj_body, 0)
    wo_copy(0).wait(); wo_copy(1).wait()
    gcol_scr[...] = jnp.broadcast_to(gw_scr[...].astype(F32).reshape(1, D), (128, D)).T

    def gate(n):
        gc = gcol_scr[...]
        for j in range(W // 128):
            xs = x_scr[n, :, j * 128:(j + 1) * 128].astype(F32)
            gs = jnp.sum((xs * gc).reshape(D // 8, 8, 128), axis=0)
            gs = jnp.broadcast_to(jnp.sum(gs, axis=0, keepdims=True), (8, 128))
            g_scr[n, :, j * 128:(j + 1) * 128] = jax.nn.sigmoid(gs)

    def qk_chunk(h, q, c, m, sub):
        kc = k_scr[h, c * CK // W, pl.ds(c * CK % W, CK), 0:DP]
        s = jnp.dot(kc, q, preferred_element_type=F32)
        s_scr[sub, pl.ds(c * CK, CK), :] = s
        mc = jnp.max(s.reshape(CK // 8, 8, W), axis=0)
        return mc if m is None else jnp.maximum(m, mc)

    def pv_chunk(h, c, m, acc, sub):
        s = s_scr[sub, pl.ds(c * CK, CK), :]
        p = jnp.exp2(s.reshape(CK // 8, 8, W) - m[None]).reshape(CK, W).astype(BF16)
        v = vt_scr[h, c * CK // W, :, pl.ds(c * CK % W, CK)]
        o = jnp.dot(v, p, preferred_element_type=F32)
        return o if acc is None else acc + o

    def unit(u):
        return u % NH, (u // NH) * NS

    def row_max(m8):
        return jnp.broadcast_to(jnp.max(m8, axis=0, keepdims=True), m8.shape)

    order = [(sub, g * GRP + j) for g in range(NC // GRP) for sub in range(NS) for j in range(GRP)]

    def step(u):
        h, q0 = unit(u)
        hn, qn = unit(u + 1)
        m_cur = row_max(m_scr[...])
        ms = [None] * NS
        accs = [None] * NS
        qs = [qt_scr[hn, qn + sub] for sub in range(NS)]
        for sub, c in order:
            accs[sub] = pv_chunk(h, c, m_cur[:, sub * W:(sub + 1) * W], accs[sub], sub)
            if c == NC - 1:
                acc_scr[h, q0 + sub] = accs[sub]
            ms[sub] = qk_chunk(hn, qs[sub], c, ms[sub], sub)
            if c == NC - 1:
                m_scr[:, pl.ds(sub * W, W)] = ms[sub]

    for sub in range(NS):
        q = qt_scr[0, sub]
        m = None
        for c in range(NC):
            m = qk_chunk(0, q, c, m, sub)
        m_scr[:, pl.ds(sub * W, W)] = m

    def body(i, carry):
        for j in range(UNROLL):
            step(i * UNROLL + j)
        return carry

    lax.fori_loop(0, (total - 1) // UNROLL, body, 0)
    for u in range((total - 1) // UNROLL * UNROLL, total - 1):
        step(u)

    def last_pv(sub):
        h, q0 = unit(total - 1)
        m_cur = row_max(m_scr[:, pl.ds(sub * W, W)])
        acc = None
        for c in range(NC):
            acc = pv_chunk(h, c, m_cur, acc, sub)
        acc_scr[h, q0 + sub] = acc
        for j in range(NCH // NS):
            gate(sub * (NCH // NS) + j)

    parts = [(n, 0, D) for n in range(NCH - 1)] + [(NCH - 1, 0, MS), (NCH - 1, MS, D)]

    def out_copy(i):
        n, lo, hi = parts[i]
        return pltpu.make_async_copy(
            out_scr.at[n, pl.ds(lo, hi - lo)], o_hbm.at[pl.ds(lo, hi - lo), pl.ds(n * W, W)], sem_o.at[i])

    def out_chunk(n):
        g = g_scr[n][0:1, :]
        rows = []
        for hh in range(NH):
            a = acc_scr[hh, n]
            gg = g if hh < H else 1.0 - g
            rows.append(a[0:DH] * (gg / a[DH:DH + 1]))
        ot = jnp.concatenate(rows, axis=0).astype(BF16)
        for i, (pn, lo, hi) in enumerate(parts):
            if pn == n:
                o = lax.dot_general(wo_scr[:, lo:hi], ot, tn, preferred_element_type=F32)
                out_scr[n, lo:hi] = o.astype(out_scr.dtype)
                out_copy(i).start()

    for sub in range(NS):
        last_pv(sub)
        out_chunk(sub)
    for n in range(NS, NCH):
        out_chunk(n)
    for i in range(len(parts)):
        out_copy(i).wait()


@jax.jit
def pallas_gated_mix__mha_block__mha_block__prompt_kernel(A_x, A_wqkv, A_wo, B_x, B_wqkv, B_wo, gate_w):
    del B_x
    _, S, D = A_x.shape
    NCH = S // W
    hbm = pl.BlockSpec(memory_space=pltpu.HBM)
    out = pl.pallas_call(
        functools.partial(_kernel, S=S, D=D),
        out_shape=jax.ShapeDtypeStruct((D, S), A_x.dtype),
        in_specs=[hbm] * 6,
        out_specs=hbm,
        scratch_shapes=[
            pltpu.VMEM((NCH, D, W), BF16),
            pltpu.VMEM((2, D, 3 * D), BF16),
            pltpu.VMEM((2 * D, D), BF16),
            pltpu.VMEM((D,), BF16),
            pltpu.VMEM((D, 128), F32),
            pltpu.VMEM((2 * H, NCH, W, 128), BF16),
            pltpu.VMEM((2 * H, NCH, DP, W), BF16),
            pltpu.VMEM((2 * H, NCH, DP, W), BF16),
            pltpu.VMEM((NCH, 8, W), F32),
            pltpu.VMEM((BQ // W, S, W), F32),
            pltpu.VMEM((8, BQ), F32),
            pltpu.VMEM((2 * H, NCH, DP, W), F32),
            pltpu.VMEM((NCH, D, W), BF16),
            pltpu.SemaphoreType.DMA((NCH,)),
            pltpu.SemaphoreType.DMA((2,)),
            pltpu.SemaphoreType.DMA((2,)),
            pltpu.SemaphoreType.DMA(()),
            pltpu.SemaphoreType.DMA((NCH + 1,)),
        ],
        compiler_params=pltpu.CompilerParams(vmem_limit_bytes=100 * 1024 * 1024),
    )(A_x[0].T, A_wqkv, B_wqkv, A_wo, B_wo, gate_w)
    return out.T[None]
```
